```python
import os as _os
_os.environ.setdefault('JAX_PLATFORMS', 'cpu')
import jax
import jax.numpy as jnp

def _softmax(x, axis=-1):
    return jax.nn.softmax(x, axis=axis)

def _gelu(x):
    return jax.nn.gelu(x, approximate=True)

def _silu(x):
    return jax.nn.silu(x)

def _sigmoid(x):
    return jax.nn.sigmoid(x)

def _layernorm(x, axis=-1, eps=1e-05):
    m = jnp.mean(x, axis=axis, keepdims=True)
    v = jnp.var(x, axis=axis, keepdims=True)
    return (x - m) / jnp.sqrt(v + eps)

def _scatter_add(tgt, idx, src, axis=0):
    return tgt.at[idx].add(src)

def _segment_sum(src, seg, n):
    return jax.ops.segment_sum(src, seg, n)

class _Rng:

    def __init__(self, key):
        self._k = key

    def _next(self):
        self._k, sub = jax.random.split(self._k)
        return sub

    def normal(self, shape):
        return jax.random.normal(self._next(), shape, dtype=jnp.bfloat16)

    def randint(self, lo, hi, shape):
        return jax.random.randint(self._next(), shape, lo, hi, dtype=jnp.int32)

    def uniform(self, shape, lo=0.0, hi=1.0):
        return jax.random.uniform(self._next(), shape, jnp.bfloat16, lo, hi)

    def permutation(self, n):
        return jax.random.permutation(self._next(), n)
kernel_name = 'gated_mix__memory_aug_recurrent_mem_tr__glu_gated_geglu__prompt'

def setup_inputs():
    _rng = _Rng(jax.random.key(int.from_bytes(__import__("os").urandom(4), "little")))
    _w = lambda a: (lambda t: t.astype(jnp.bfloat16) if jnp.issubdtype(t.dtype, jnp.floating) else t)(jnp.asarray(a))

    def _A_setup():
        B, S, Dm = (1, 2048, 640)
        H, Dh = (32, 128)
        M, seg = (8, 32)
        seg = min(seg, S)
        S = S // seg * seg
        return {'x': _w((lambda *s: _rng.normal(s) * 0.05)(B, S, Dm)), 'mem0': _w((lambda *s: _rng.normal(s) * 0.4)(B, M, Dm)), 'Wq': _w((lambda *s: _rng.normal(s) * 3.2)(Dm, H, Dh) * Dm ** (-0.5)), 'Wk': _w((lambda *s: _rng.normal(s) * 3.2)(Dm, H, Dh) * Dm ** (-0.5)), 'Wv': _w((lambda *s: _rng.normal(s) * 0.4)(Dm, H, Dh) * Dm ** (-0.5)), 'Wo': _w((lambda *s: _rng.normal(s) * 0.4)(H, Dh, Dm) * (H * Dh) ** (-0.5)), 'seg_len': seg}
    _A_in = _A_setup()

    def _B_setup():
        B, S, Dm, Df = (1, 2048, 640, 1728)
        return {'x': _w((lambda *s: _rng.normal(s) * 0.05)(B, S, Dm)), 'w_gate': _w((lambda *s: _rng.normal(s) * 1.6)(Dm, Df) * Dm ** (-0.5)), 'w_up': _w((lambda *s: _rng.normal(s) * 1.6)(Dm, Df) * Dm ** (-0.5)), 'w_down': _w((lambda *s: _rng.normal(s) * 1.6)(Df, Dm) * Df ** (-0.5))}
    _B_in = _B_setup()
    return {'A_x': _A_in['x'], 'A_mem0': _A_in['mem0'], 'A_Wq': _A_in['Wq'], 'A_Wk': _A_in['Wk'], 'A_Wv': _A_in['Wv'], 'A_Wo': _A_in['Wo'], 'A_seg_len': _A_in['seg_len'], 'B_x': _B_in['x'], 'B_w_gate': _B_in['w_gate'], 'B_w_up': _B_in['w_up'], 'B_w_down': _B_in['w_down'], 'gate_w': _w((lambda *s: _rng.normal(s) * 0.05)(640) * 16.0)}

def reference(A_x, A_mem0, A_Wq, A_Wk, A_Wv, A_Wo, A_seg_len, B_x, B_w_gate, B_w_up, B_w_down, gate_w):

    def _A_ref(x, mem0, Wq, Wk, Wv, Wo, seg_len):
        B, S, Dm = x.shape
        H, Dh = (Wq.shape[1], Wq.shape[2])
        M = mem0.shape[1]
        scale = Dh ** (-0.5)
        n_seg = S // seg_len
        L = M + seg_len
        idx = jnp.arange(L)
        mask = (idx[:, None] < M) | (idx[:, None] >= idx[None, :])
        mem = mem0
        outs = []
        for s in range(n_seg):
            xs = x[:, s * seg_len:(s + 1) * seg_len, :].copy()
            h = jnp.concatenate([mem, xs], axis=1)
            q = jnp.einsum('btd,dhe->bhte', h, Wq)
            k = jnp.einsum('btd,dhe->bhte', h, Wk)
            v = jnp.einsum('btd,dhe->bhte', h, Wv)
            scores = jnp.einsum('bhqe,bhke->bhqk', q, k) * scale
            scores = jnp.where(mask[None, None], scores, -1000000000.0)
            p = _softmax(scores, axis=-1)
            o = jnp.einsum('bhqk,bhke->bhqe', p, v)
            o = jnp.einsum('bhte,hed->btd', o, Wo)
            mem = o[:, :M, :].copy()
            outs.append(o[:, M:, :])
        return jnp.concatenate(outs, axis=1)

    def _B_ref(x, w_gate, w_up, w_down):
        g = jnp.einsum('bsd,df->bsf', x, w_gate)
        u = jnp.einsum('bsd,df->bsf', x, w_up)
        h = _gelu(g) * u
        return jnp.einsum('bsf,fd->bsd', h, w_down)
    x = A_x
    g = _sigmoid((x * gate_w).sum(-1, keepdims=True))
    a = _A_ref(x, A_mem0, A_Wq, A_Wk, A_Wv, A_Wo, A_seg_len)
    b = _B_ref(x, B_w_gate, B_w_up, B_w_down)
    return g * a + (1 - g) * b
```

```python
import functools

import jax
import jax.numpy as jnp
import jax.experimental.pallas as pl
import jax.experimental.pallas.tpu as pltpu

F32 = jnp.float32
BF16 = jnp.bfloat16
U32 = jnp.uint32


def _dot(a, b):
    return jnp.dot(a, b, preferred_element_type=F32)


def _dot_nt(a, b):
    return jax.lax.dot_general(a, b, (((1,), (1,)), ((), ())),
                               preferred_element_type=F32)


def _kernel(x_ref, mem0_ref, wq_ref, wk_ref, wv_ref, wo_ref, wg_ref, wu_ref,
            wd_ref, gw_ref, out_ref,
            wqkv_s, u_s, bb_s, gg_s, mem_s, stq_s, sto_s, oa_s,
            *, S, D, H, E, M, SEG, DF):
    L = M + SEG
    P = 17
    scale = float(E) ** -0.5

    for wi, w_ref in enumerate((wq_ref, wk_ref, wv_ref)):
        CH = 64
        for d0 in range(0, D, CH):
            u = pltpu.bitcast(w_ref[d0:d0 + CH], U32)
            for d in range(CH):
                u_s[(d0 + d) * P:(d0 + d) * P + H // 2, :] = u[d]
        for j in range(H // 2):
            a = u_s[pl.ds(j, D // 2, stride=2 * P), :]
            b = u_s[pl.ds(P + j, D // 2, stride=2 * P), :]
            lo = (a & U32(0xFFFF)) | (b << 16)
            hi = (a >> 16) | (b & U32(0xFFFF0000))
            wqkv_s[wi, 2 * j] = pltpu.bitcast(lo, BF16)
            wqkv_s[wi, 2 * j + 1] = pltpu.bitcast(hi, BF16)

    TB = 256

    def ffn_body(i, c):
        r0 = pl.multiple_of(i * TB, TB)
        xb = x_ref[pl.ds(r0, TB), :]
        g = _dot(xb, wg_ref[...])
        u = _dot(xb, wu_ref[...])
        h = (jax.nn.gelu(g, approximate=True) * u).astype(BF16)
        b = _dot(h, wd_ref[...])
        z = jnp.sum(xb.astype(F32) * gw_ref[...].astype(F32), axis=-1,
                    keepdims=True)
        gt = jax.nn.sigmoid(z)
        bb_s[pl.ds(r0, TB), :] = (1.0 - gt) * b
        gg_s[pl.ds(r0, TB), :] = jnp.broadcast_to(gt, (TB, 128))
        return c

    jax.lax.fori_loop(0, S // TB, ffn_body, 0)

    mem_s[...] = mem0_ref[...].astype(F32)

    ri = jax.lax.broadcasted_iota(jnp.int32, (2 * L, 2 * L), 0)
    ci = jax.lax.broadcasted_iota(jnp.int32, (2 * L, 2 * L), 1)
    rhi = ri >= L
    chi = ci >= L
    rr = jnp.where(rhi, ri - L, ri)
    cc = jnp.where(chi, ci - L, ci)
    mask = (rhi == chi) & ((rr < M) | (rr >= cc))

    def attn_pair(q2, k2, v2):
        s = _dot_nt(q2.astype(BF16), k2.astype(BF16)) * scale
        s = jnp.where(mask, s, -1000000000.0)
        m = jnp.max(s, axis=-1, keepdims=True)
        p = jnp.exp(s - m)
        l = jnp.sum(p, axis=-1, keepdims=True)
        p = (p * (1.0 / l)).astype(BF16)
        return _dot(p, v2.astype(BF16))

    def seg_body(j, c):
        r0 = pl.multiple_of(j * 2 * SEG, 2 * SEG)
        xf = x_ref[pl.ds(r0, 2 * SEG), :].astype(F32)

        ha = jnp.concatenate([mem_s[...], xf[0:L]], axis=0).astype(BF16)
        for hp in range(H // 2):
            t = []
            for wi in range(3):
                y0 = _dot(ha, wqkv_s[wi, 2 * hp])
                y1 = _dot(ha, wqkv_s[wi, 2 * hp + 1])
                stq_s[wi, 2 * hp] = y0[L:L + M]
                stq_s[wi, 2 * hp + 1] = y1[L:L + M]
                t.append(jnp.concatenate([y0[0:L], y1[0:L]], axis=0))
            o = attn_pair(*t)
            o0, o1 = o[0:L], o[L:2 * L]
            sto_s[2 * hp] = o0[SEG:L]
            sto_s[2 * hp + 1] = o1[SEG:L]
            oa_s[0:SEG, (2 * hp) * E:(2 * hp + 1) * E] = o0[0:SEG].astype(BF16)
            oa_s[0:SEG, (2 * hp + 1) * E:(2 * hp + 2) * E] = (
                o1[0:SEG].astype(BF16))
        acc_a = _dot(oa_s[0:SEG, :], wo_ref[...])
        mem_b = acc_a[0:M]

        hb = jnp.concatenate([mem_b, xf[L:2 * SEG]], axis=0).astype(BF16)
        for hp in range(H // 2):
            t = []
            for wi in range(3):
                y0 = _dot(hb, wqkv_s[wi, 2 * hp])
                y1 = _dot(hb, wqkv_s[wi, 2 * hp + 1])
                t.append(jnp.concatenate(
                    [y0[0:M], stq_s[wi, 2 * hp], y0[M:SEG],
                     y1[0:M], stq_s[wi, 2 * hp + 1], y1[M:SEG]], axis=0))
            o = attn_pair(*t)
            oa_s[:, (2 * hp) * E:(2 * hp + 1) * E] = jnp.concatenate(
                [o[0:L], sto_s[2 * hp]], axis=0).astype(BF16)
            oa_s[:, (2 * hp + 1) * E:(2 * hp + 2) * E] = jnp.concatenate(
                [o[L:2 * L], sto_s[2 * hp + 1]], axis=0).astype(BF16)
        acc_b = _dot(oa_s[...], wo_ref[...])
        mem_s[...] = acc_b[0:M]

        a = jnp.concatenate([acc_a[M:SEG], acc_b[L:L + M], acc_b[M:L]], axis=0)
        gt = gg_s[pl.ds(r0, 2 * SEG), :]
        gt = jnp.concatenate([gt] * (D // 128), axis=1)
        out_ref[pl.ds(r0, 2 * SEG), :] = (
            gt * a + bb_s[pl.ds(r0, 2 * SEG), :]).astype(out_ref.dtype)
        return c

    jax.lax.fori_loop(0, S // (2 * SEG), seg_body, 0)


@jax.jit
def pallas_gated_mix__memory_aug_recurrent_mem_tr__glu_gated_geglu__prompt_kernel(
    A_x: jax.Array,
    A_mem0: jax.Array,
    A_Wq: jax.Array,
    A_Wk: jax.Array,
    A_Wv: jax.Array,
    A_Wo: jax.Array,
    A_seg_len: jax.Array,
    B_x: jax.Array,
    B_w_gate: jax.Array,
    B_w_up: jax.Array,
    B_w_down: jax.Array,
    gate_w: jax.Array,
):
    B, S, D = A_x.shape
    H, E = A_Wq.shape[1], A_Wq.shape[2]
    M = A_mem0.shape[1]
    DF = B_w_gate.shape[1]
    SEG = 32
    assert B == 1 and M == 8 and S % (2 * SEG) == 0

    kern = functools.partial(_kernel, S=S, D=D, H=H, E=E, M=M, SEG=SEG, DF=DF)
    out = pl.pallas_call(
        kern,
        out_shape=jax.ShapeDtypeStruct((S, D), A_x.dtype),
        scratch_shapes=[
            pltpu.VMEM((3, H, D, E), BF16),
            pltpu.VMEM((D * 17, E), U32),
            pltpu.VMEM((S, D), F32),
            pltpu.VMEM((S, 128), F32),
            pltpu.VMEM((M, D), F32),
            pltpu.VMEM((3, H, M, E), F32),
            pltpu.VMEM((H, M, E), F32),
            pltpu.VMEM((SEG + 2 * M, H * E), BF16),
        ],
        compiler_params=pltpu.CompilerParams(
            vmem_limit_bytes=110 * 1024 * 1024),
    )(
        A_x.reshape(S, D), A_mem0.reshape(M, D), A_Wq, A_Wk, A_Wv,
        A_Wo.reshape(H * E, D), B_w_gate, B_w_up, B_w_down,
        gate_w.reshape(1, D),
    )
    return out.reshape(B, S, D)
```

```python
import functools

import jax
import jax.numpy as jnp
import jax.experimental.pallas as pl
import jax.experimental.pallas.tpu as pltpu

F32 = jnp.float32
BF16 = jnp.bfloat16
U32 = jnp.uint32
PH_ = 321
ANCH = ((0, 0), (128, 128), (0, 384), (128, 512))


def _mk_sched(cfg):
    NP = 16
    dp, ds = cfg.get('dp', 3), cfg.get('ds', 1)
    fill = {}
    for pos, f in cfg.get('fill', []):
        fill.setdefault(str(pos), []).append(tuple(f))
    early = {int(k): v for k, v in cfg.get('early_w', {}).items()}
    out = list(fill.get('start', []))
    for t in range(NP):
        out.append(('q', t))
        if t >= dp:
            out.append(('p', t - dp))
        if t >= ds:
            out.append(('s', t - ds))
        if t in early:
            out.append(('w',) + tuple(early[t]))
        out += fill.get(str(t), [])
    for k, op in enumerate(cfg['tail']):
        out.append(tuple(op))
        out += fill.get('t%d' % k, [])
    return out


_T1 = dict(early_w={'14': [0, 2]},
           tail=[['w', 2, 5], ['p', 13], ['s', 15], ['w', 5, 8], ['p', 14],
                 ['w', 8, 12], ['p', 15], ['w', 12, 15], ['w', 15, 16]])
_T3 = dict(early_w={'13': [0, 1], '14': [1, 2]}, tail=_T1['tail'])
_T6 = dict(early_w={'12': [0, 2], '14': [2, 4]},
           tail=[['w', 4, 6], ['p', 13], ['s', 15], ['w', 6, 9], ['p', 14],
                 ['w', 9, 12], ['p', 15], ['w', 12, 15], ['w', 15, 16]])
_CFG = dict(
    fa=dict(_T6, fill=[['t8', ['g', 0]]]),
    fb=dict(_T1,
            fill=[[0, ['u', 0]], [2, ['g', 1]], [4, ['u', 1]], [7, ['d', 0]],
                  [9, ['d', 1]], [11, ['d', 2]], [13, ['d', 3]],
                  [15, ['d', 4]]]),
    na=_T3,
    nb=_T3,
)
SCHED_F = (_mk_sched(_CFG['fa']), _mk_sched(_CFG['fb']))
SCHED_N = (_mk_sched(_CFG['na']), _mk_sched(_CFG['nb']))


def _dot(a, b):
    return jnp.dot(a, b, preferred_element_type=F32)


def _dot_nt(a, b):
    return jax.lax.dot_general(a, b, (((1,), (1,)), ((), ())),
                               preferred_element_type=F32)


def _kernel(x_hbm, mem0_ref, wq_hbm, wk_hbm, wv_hbm, wo_hbm, wgt_hbm, wut_hbm,
            wd_hbm, gw_ref, out_hbm,
            x_s, wraw_s, wor_s, wgt_s, wut_s, wd_s, wqkv_s, bb_s,
            mem_s, stq_s, sto_s, oa_s, out_s, sems, osem,
            *, S, D, H, E, M, SEG, DF, DFP):
    L = M + SEG
    PH = PH_
    NP = H // 2
    scale = float(E) ** -0.5
    TB = 256
    S0 = 5 * TB
    TF = 192
    CW = 256
    NC = DFP // CW

    T0 = 2 * TB
    GCH = (0, 512, 1280, DF)

    def xcopy(a, b, k):
        return pltpu.make_async_copy(x_hbm.at[pl.ds(a, b - a)],
                                     x_s.at[pl.ds(a, b - a)], sems.at[k])

    cp_x0 = xcopy(0, T0, 0)
    cp_wg = [pltpu.make_async_copy(
        wgt_hbm.at[pl.ds(GCH[k], GCH[k + 1] - GCH[k])],
        wgt_s.at[pl.ds(GCH[k], GCH[k + 1] - GCH[k])], sems.at[1 + k])
        for k in range(3)]
    cp_wu = pltpu.make_async_copy(wut_hbm, wut_s.at[pl.ds(0, DF)], sems.at[4])
    cp_wd = pltpu.make_async_copy(wd_hbm, wd_s.at[pl.ds(0, DF)], sems.at[5])
    cp_x1 = xcopy(T0, S0, 6)
    cp_w = [pltpu.make_async_copy(w, wraw_s.at[i], sems.at[7 + i])
            for i, w in enumerate((wq_hbm, wk_hbm, wv_hbm))]
    cp_wo = pltpu.make_async_copy(wo_hbm, wor_s, sems.at[10])
    cp_x2 = xcopy(S0, S, 11)
    DFT = DFP - 128
    assert DFP - DF == DF - DFT == 64
    cp_wm = pltpu.make_async_copy(wut_hbm.at[pl.ds(DFT, DF - DFT)],
                                  wgt_s.at[pl.ds(DF, DFP - DF)], sems.at[12])
    cp_x0.start()
    for c in cp_wg:
        c.start()
    cp_wm.start()

    zpad = jnp.zeros((DFP - DF, D), BF16)
    wut_s[DF:DFP, :] = zpad
    wd_s[DF:DFP, :] = zpad
    bb_s[S0:S, :] = jnp.zeros((S - S0, D), F32)
    mem_s[...] = mem0_ref[...].astype(F32)

    def geglu(g, u):
        return (jax.nn.gelu(g, approximate=True) * u).astype(BF16)

    def geglu_mixed(t):
        lane = jax.lax.broadcasted_iota(jnp.int32, t.shape, 1)
        hm = jax.nn.gelu(t, approximate=True) * pltpu.roll(t, 64, 1)
        return jnp.where(lane < 64, hm, 0.0).astype(BF16)

    cp_x0.wait()
    cp_wg[0].wait()
    cp_wu.start()
    cp_wd.start()
    cp_x1.start()
    for c in cp_w:
        c.start()
    cp_wo.start()
    cp_x2.start()
    xb = x_s[0:T0, :]
    gparts = [_dot_nt(xb, wgt_s[GCH[0]:GCH[1], :])]
    cp_wg[1].wait()
    gparts.append(_dot_nt(xb, wgt_s[GCH[1]:GCH[2], :]))
    cp_wg[2].wait()
    cp_wm.wait()
    gparts.append(_dot_nt(xb, wgt_s[GCH[2]:DFP, :]))
    g = jnp.concatenate(gparts, axis=1)
    cp_wu.wait()
    h0 = geglu(g[:, 0:1024], _dot_nt(xb, wut_s[0:1024, :]))
    cp_wd.wait()
    h1 = geglu(g[:, 1024:DFT], _dot_nt(xb, wut_s[1024:DFT, :]))
    h = jnp.concatenate([h0, h1, geglu_mixed(g[:, DFT:DFP])], axis=1)
    bb_s[0:T0, :] = _dot(h, wd_s[...])
    cp_x1.wait()

    def ffn_body(i, c):
        pltpu.make_async_copy(wq_hbm, wraw_s.at[i], sems.at[7 + i]).wait()
        r0 = pl.multiple_of(T0 + i * TB, TB)
        xb = x_s[pl.ds(r0, TB), :]

        NPC = 64
        DP = D // NPC
        todo = list(range(NPC))

        def relayout_piece(k):
            uu = pltpu.bitcast(wraw_s[i, k * DP:(k + 1) * DP], U32)
            t = None
            for r in range(DP // 2):
                a = uu[2 * r]
                b = uu[2 * r + 1]
                rr = k * DP // 2 + r
                lo = (a & U32(0xFFFF)) | (b << 16)
                hi = (a >> 16) | (b & U32(0xFFFF0000))
                wqkv_s[i, pl.ds(rr, H // 2, stride=2 * PH), :] = lo
                wqkv_s[i, pl.ds(PH + rr, H // 2, stride=2 * PH), :] = hi
                t = (lo | hi) if t is None else (t | lo | hi)
            t = pltpu.bitcast(t[0:8] | t[8:16], jnp.int32)
            return pltpu.bitcast(jnp.minimum(t & 1, 0), U32)

        def anchor_at(m, ra, ca):
            if not todo:
                return m
            z = relayout_piece(todo.pop(0))
            blk = pltpu.bitcast(
                pltpu.bitcast(m[ra:ra + 16, ca:ca + 128], U32) | z, BF16)
            cols = [m[ra:ra + 16, :ca], blk, m[ra:ra + 16, ca + 128:]]
            mid = jnp.concatenate([q for q in cols if q.shape[1]], axis=1)
            rows = [m[:ra], mid, m[ra + 16:]]
            return jnp.concatenate([q for q in rows if q.shape[0]], axis=0)

        def anchored(m, first=False):
            if first:
                return m
            for ra, ca in ANCH:
                m = anchor_at(m, ra, ca)
            return m

        hs = []
        for n in range(NC):
            gg = _dot_nt(anchored(xb, n == 0), wgt_s[n * CW:(n + 1) * CW, :])
            if n < NC - 1:
                uu = _dot_nt(anchored(xb), wut_s[n * CW:(n + 1) * CW, :])
                hs.append(geglu(gg, uu))
            else:
                uu = _dot_nt(anchored(xb), wut_s[n * CW:DFT, :])
                hs.append(geglu(gg[:, 0:CW - 128], uu))
                hs.append(geglu_mixed(gg[:, CW - 128:CW]))
        h = jnp.concatenate(hs, axis=1)
        for n in range(D // 128):
            bb_s[pl.ds(r0, TB), n * 128:(n + 1) * 128] = _dot(
                anchored(h), wd_s[:, n * 128:(n + 1) * 128])
        assert not todo
        return c

    jax.lax.fori_loop(0, 3, ffn_body, 0)

    cp_wo.wait()
    cp_x2.wait()

    ri = jax.lax.broadcasted_iota(jnp.int32, (2 * L, 2 * L), 0)
    ci = jax.lax.broadcasted_iota(jnp.int32, (2 * L, 2 * L), 1)
    rhi = ri >= L
    chi = ci >= L
    rr = jnp.where(rhi, ri - L, ri)
    cc = jnp.where(chi, ci - L, ci)
    mask = (rhi == chi) & ((rr < M) | (rr >= cc))
    fill = jnp.where(rhi == chi, -1000000000.0, -jnp.inf).astype(F32)

    def w_qkv(wi, h):
        return pltpu.bitcast(wqkv_s[wi, h * PH:h * PH + D // 2, :], BF16)

    def softmax_pv(s, v2):
        s = jnp.where(mask, s * scale, fill)
        m = jnp.max(s, axis=-1, keepdims=True)
        p = jnp.exp(s - m)
        l = jnp.sum(p, axis=-1, keepdims=True)
        r = pl.reciprocal(l, approx=True)
        r = r * (2.0 - l * r)
        return _dot((p * r).astype(BF16), v2)

    def wo_part(rows, p0, p1):
        lhs = pltpu.bitcast(oa_s[0:rows // 2, p0 * 2 * E:p1 * 2 * E], BF16)
        rhs = wor_s[p0 * 2 * E:p1 * 2 * E, :]
        return _dot(lhs, rhs)

    def substep(hmat, is_a, sched, fillers):
        qkv = {}
        sc = {}

        def do_qkv(t):
            r = []
            for wi in range(3):
                y0 = _dot(hmat, w_qkv(wi, 2 * t))
                y1 = _dot(hmat, w_qkv(wi, 2 * t + 1))
                if is_a:
                    stq_s[wi, 2 * t] = y0[L:L + M]
                    stq_s[wi, 2 * t + 1] = y1[L:L + M]
                    z = jnp.concatenate([y0[0:L], y1[0:L]], axis=0)
                else:
                    z = jnp.concatenate(
                        [y0[0:M], stq_s[wi, 2 * t], y0[M:SEG],
                         y1[0:M], stq_s[wi, 2 * t + 1], y1[M:SEG]], axis=0)
                r.append(z.astype(BF16))
            qkv[t] = r

        def do_s(t):
            sc[t] = _dot_nt(qkv[t][0], qkv[t][1])

        def do_pv(t):
            o = softmax_pv(sc.pop(t), qkv.pop(t)[2])
            for k in range(2):
                h = 2 * t + k
                ok = o[k * L:(k + 1) * L]
                if is_a:
                    sto_s[h] = ok[SEG:L]
                    ob = ok[0:SEG].astype(BF16)
                    oa_s[0:SEG // 2, h * E:(h + 1) * E] = pltpu.bitcast(ob, U32)
                else:
                    ob = jnp.concatenate([ok, sto_s[h]], axis=0).astype(BF16)
                    oa_s[:, h * E:(h + 1) * E] = pltpu.bitcast(ob, U32)

        rows = SEG if is_a else SEG + 2 * M
        acc = None
        for op in sched:
            kind = op[0]
            if kind == 'q':
                do_qkv(op[1])
            elif kind == 's':
                do_s(op[1])
            elif kind == 'p':
                do_pv(op[1])
            elif kind == 'w':
                part = wo_part(rows, op[1], op[2])
                acc = part if acc is None else acc + part
            elif fillers:
                fillers[kind](op[1])
        return acc

    def seg_body(j, c, with_ffn):
        r0 = pl.multiple_of(j * 2 * SEG, 2 * SEG)
        xf = x_s[pl.ds(r0, 2 * SEG), :].astype(F32)

        z = jnp.sum(xf * gw_ref[...].astype(F32).reshape(1, D), axis=-1, keepdims=True)
        gt = jax.nn.sigmoid(z)
        bpart = (1.0 - gt) * bb_s[pl.ds(r0, 2 * SEG), :]

        fills = {}
        sa, sb = SCHED_F if with_ffn else SCHED_N
        if with_ffn:
            fr0 = pl.multiple_of(S0 + (j // NC) * TF, 64)
            fc0 = pl.multiple_of((j % NC) * CW, CW)
            hs = []

            gs = {}

            def gate(k):
                xg = x_s[pl.ds(fr0, TF), :]
                c0 = pl.multiple_of(fc0 + k * 128, 128)
                gs[k] = _dot_nt(xg, wgt_s[pl.ds(c0, 128), :])

            def up(k):
                xg = x_s[pl.ds(fr0, TF), :]
                c0 = pl.multiple_of(fc0 + k * 128, 128)
                u = _dot_nt(xg, wut_s[pl.ds(c0, 128), :])
                hs.append(geglu(gs.pop(k), u))

            def down(n):
                hcat = jnp.concatenate(hs, axis=1)
                w = wd_s[pl.ds(fc0, CW), n * 128:(n + 1) * 128]
                bb_s[pl.ds(fr0, TF), n * 128:(n + 1) * 128] += _dot(hcat, w)

            fills = dict(g=gate, u=up, d=down)

        ha = jnp.concatenate([mem_s[...], xf[0:L]], axis=0).astype(BF16)
        acc_a = substep(ha, True, sa, fills)
        hb = jnp.concatenate([acc_a[0:M], xf[L:2 * SEG]],
                             axis=0).astype(BF16)
        acc_b = substep(hb, False, sb, fills)
        mem_s[...] = acc_b[0:M]

        a = jnp.concatenate([acc_a[M:SEG], acc_b[L:L + M], acc_b[M:L]], axis=0)
        out_s[pl.ds(r0, 2 * SEG), :] = (gt * a + bpart).astype(out_s.dtype)
        pltpu.make_async_copy(out_s.at[pl.ds(r0, 2 * SEG)],
                              out_hbm.at[pl.ds(r0, 2 * SEG)], osem).start()
        return c

    n_it = S // (2 * SEG)
    n_ffn = ((S - S0) // TF) * NC
    jax.lax.fori_loop(0, n_ffn, functools.partial(seg_body, with_ffn=True), 0)
    jax.lax.fori_loop(n_ffn, n_it,
                      functools.partial(seg_body, with_ffn=False), 0)
    pltpu.make_async_copy(out_s, out_hbm, osem).wait()


@jax.jit
def pallas_gated_mix__memory_aug_recurrent_mem_tr__glu_gated_geglu__prompt_kernel(
    A_x: jax.Array,
    A_mem0: jax.Array,
    A_Wq: jax.Array,
    A_Wk: jax.Array,
    A_Wv: jax.Array,
    A_Wo: jax.Array,
    A_seg_len: jax.Array,
    B_x: jax.Array,
    B_w_gate: jax.Array,
    B_w_up: jax.Array,
    B_w_down: jax.Array,
    gate_w: jax.Array,
):
    B, S, D = A_x.shape
    H, E = A_Wq.shape[1], A_Wq.shape[2]
    M = A_mem0.shape[1]
    DF = B_w_gate.shape[1]
    DFP = -(-DF // 256) * 256
    SEG = 32
    assert B == 1 and M == 8 and S % 512 == 0

    kern = functools.partial(_kernel, S=S, D=D, H=H, E=E, M=M, SEG=SEG, DF=DF,
                             DFP=DFP)
    hbm = pl.BlockSpec(memory_space=pl.ANY)
    vm = pl.BlockSpec(memory_space=pltpu.VMEM)
    out = pl.pallas_call(
        kern,
        out_shape=jax.ShapeDtypeStruct((S, D), A_x.dtype),
        in_specs=[hbm, vm, hbm, hbm, hbm, hbm, hbm, hbm, hbm, vm],
        out_specs=hbm,
        scratch_shapes=[
            pltpu.VMEM((S, D), BF16),
            pltpu.VMEM((3, D, H, E), BF16),
            pltpu.VMEM((H * E, D), BF16),
            pltpu.VMEM((DFP, D), BF16),
            pltpu.VMEM((DFP, D), BF16),
            pltpu.VMEM((DFP, D), BF16),
            pltpu.VMEM((3, H * PH_, E), U32),
            pltpu.VMEM((S, D), F32),
            pltpu.VMEM((M, D), F32),
            pltpu.VMEM((3, H, M, E), F32),
            pltpu.VMEM((H, M, E), F32),
            pltpu.VMEM(((SEG + 2 * M) // 2, H * E), U32),
            pltpu.VMEM((S, D), BF16),
            pltpu.SemaphoreType.DMA((13,)),
            pltpu.SemaphoreType.DMA,
        ],
        compiler_params=pltpu.CompilerParams(
            vmem_limit_bytes=110 * 1024 * 1024),
    )(
        A_x.reshape(S, D), A_mem0.reshape(M, D), A_Wq, A_Wk, A_Wv,
        A_Wo.reshape(H * E, D), B_w_gate.T, B_w_up.T, B_w_down,
        gate_w,
    )
    return out.reshape(B, S, D)
```

```python
import functools

import jax
import jax.numpy as jnp
import jax.experimental.pallas as pl
import jax.experimental.pallas.tpu as pltpu

F32 = jnp.float32
BF16 = jnp.bfloat16
U32 = jnp.uint32
PH_ = 321
ANCH = ((0, 0), (128, 128), (0, 384), (128, 512))


def _mk_sched(cfg):
    NP = 16
    dp, ds = cfg.get('dp', 3), cfg.get('ds', 1)
    fill = {}
    for pos, f in cfg.get('fill', []):
        fill.setdefault(str(pos), []).append(tuple(f))
    early = {int(k): v for k, v in cfg.get('early_w', {}).items()}
    out = list(fill.get('start', []))
    for t in range(NP):
        out.append(('q', t))
        if t >= dp:
            out.append(('p', t - dp))
        if t >= ds:
            out.append(('s', t - ds))
        if t in early:
            out.append(('w',) + tuple(early[t]))
        out += fill.get(str(t), [])
    for k, op in enumerate(cfg['tail']):
        out.append(tuple(op))
        out += fill.get('t%d' % k, [])
    return out


_T = dict(
    T1=dict(early_w={'14': [0, 2]},
            tail=[['w', 2, 5], ['p', 13], ['s', 15], ['w', 5, 8], ['p', 14],
                  ['w', 8, 12], ['p', 15], ['w', 12, 15], ['w', 15, 16]]),
    T3=dict(early_w={'13': [0, 1], '14': [1, 2]},
            tail=[['w', 2, 5], ['p', 13], ['s', 15], ['w', 5, 8], ['p', 14],
                  ['w', 8, 12], ['p', 15], ['w', 12, 15], ['w', 15, 16]]),
    T6=dict(early_w={'12': [0, 2], '14': [2, 4]},
            tail=[['w', 4, 6], ['p', 13], ['s', 15], ['w', 6, 9], ['p', 14],
                  ['w', 9, 12], ['p', 15], ['w', 12, 15], ['w', 15, 16]]),
)
_CFG = [
    ['T1', [[4, ['g', 0]], [8, ['u', 0]], ['t7', ['g', 1]], ['t8', ['u', 1]]]],
    ['T1', [[2, ['g', 2]], [5, ['u', 2]], [8, ['g', 3]], [11, ['u', 3]],
            ['t7', ['g', 4]], ['t8', ['u', 4]]]],
    ['T1', [[2, ['g', 5]], [4, ['u', 5]], [6, ['g', 6]], [8, ['u', 6]],
            ['t7', ['d', 0]], ['t8', ['d', 1]]]],
    ['T1', [[2, ['d', 2]], [5, ['d', 3]], [8, ['d', 4]], [10, ['c', 0]]]],
]
SCHED = [_mk_sched(dict(_T[t], fill=f)) for t, f in _CFG]


def _dot(a, b):
    return jnp.dot(a, b, preferred_element_type=F32)


def _dot_nt(a, b):
    return jax.lax.dot_general(a, b, (((1,), (1,)), ((), ())),
                               preferred_element_type=F32)


def _kernel(x_hbm, mem0_ref, wq_hbm, wk_hbm, wv_hbm, wo_hbm, wgt_hbm, wut_hbm,
            wd_hbm, gw_ref, out_hbm,
            x_s, wraw_s, wor_s, wgt_s, wut_s, wd_s, wqkv_s, bb_s, g_s,
            mem_s, stq_s, sto_s, oa_s, out_s, sems, wsems, osem,
            *, S, D, H, E, M, SEG, DF, DFP):
    L = M + SEG
    PH = PH_
    scale = float(E) ** -0.5
    TB = 256
    NB0 = 5
    S0 = NB0 * TB
    CW = 256
    NC = DFP // CW
    DFT = DFP - 128
    assert DFP - DF == DF - DFT == 64
    WC = 3 * D // NB0

    GCH = (0, 256, 768, DF)

    def xcopy(a, b, k):
        return pltpu.make_async_copy(x_hbm.at[pl.ds(a, b - a)],
                                     x_s.at[pl.ds(a, b - a)], sems.at[k])

    NT0 = 2
    T0 = NT0 * TB
    STG = 1
    cp_x0 = xcopy(0, T0, 0)
    cp_wg = [pltpu.make_async_copy(
        wgt_hbm.at[pl.ds(GCH[k], GCH[k + 1] - GCH[k])],
        wgt_s.at[pl.ds(GCH[k], GCH[k + 1] - GCH[k])], sems.at[1 + k])
        for k in range(3)]
    cp_wm = pltpu.make_async_copy(wut_hbm.at[pl.ds(DFT, DF - DFT)],
                                  wgt_s.at[pl.ds(DF, DFP - DF)], sems.at[4])
    cp_x1 = xcopy(T0, S0, 5)
    cp_wu = pltpu.make_async_copy(wut_hbm, wut_s.at[pl.ds(0, DF)], sems.at[6])
    cp_wd = pltpu.make_async_copy(wd_hbm, wd_s.at[pl.ds(0, DF)], sems.at[7])
    cp_w = []
    for c in range(NB0):
        a = c * WC
        cp_w.append([])
        while a < (c + 1) * WC:
            wi = a // D
            b = min((c + 1) * WC, (wi + 1) * D)
            cp_w[c].append(pltpu.make_async_copy(
                (wq_hbm, wk_hbm, wv_hbm)[wi].at[pl.ds(a - wi * D, b - a)],
                wraw_s.at[pl.ds(a, b - a)], wsems.at[c]))
            a = b

    def start_when(cond, cps):
        @pl.when(cond)
        def _():
            for cp in cps:
                cp.start()
    cp_wo = pltpu.make_async_copy(wo_hbm, wor_s, sems.at[8])
    cp_x2 = xcopy(S0, S, 9)
    cp_x0.start()
    cp_wg[0].start()
    if STG == 0:
        cp_wg[1].start()
        cp_wg[2].start()
        cp_wm.start()
        cp_x1.start()
    if STG == 1:
        cp_wg[1].start()

    zpad = jnp.zeros((DFP - DF, D), BF16)
    wut_s[DF:DFP, :] = zpad
    wd_s[DF:DFP, :] = zpad
    bb_s[S0:S, :] = jnp.zeros((S - S0, D), F32)
    mem_s[...] = mem0_ref[...].astype(F32)

    def gelu(g):
        return jax.nn.gelu(g, approximate=True)

    def gate_act(g):
        t = g[:, -128:]
        lane = jax.lax.broadcasted_iota(jnp.int32, t.shape, 1)
        hm = jnp.where(lane < 64, gelu(t) * pltpu.roll(t, 64, 1), 0.0)
        return jnp.concatenate([gelu(g[:, :-128]), hm], axis=1)

    if STG == 2:
        cp_wg[1].start()
    cp_x0.wait()
    cp_wg[0].wait()
    if STG == 0:
        cp_wu.start()
        cp_wd.start()
    else:
        cp_wg[2].start()
        cp_wm.start()
        cp_x1.start()
    xb = x_s[0:T0, :]
    g_s[0:T0, GCH[0]:GCH[1]] = gelu(_dot_nt(xb, wgt_s[GCH[0]:GCH[1], :]))
    cp_wg[1].wait()
    if STG:
        cp_wu.start()
    g_s[0:T0, GCH[1]:GCH[2]] = gelu(_dot_nt(xb, wgt_s[GCH[1]:GCH[2], :]))
    cp_wg[2].wait()
    cp_wm.wait()
    if STG:
        cp_wd.start()
    if NT0 == 2:
        for cp in cp_w[0]:
            cp.start()
    g_s[0:T0, GCH[2]:DFP] = gate_act(_dot_nt(xb, wgt_s[GCH[2]:DFP, :]))
    cp_x1.wait()

    def gate_body(i, c):
        for k in range(NT0, NB0):
            start_when(i == k, cp_w[k - 1])
        r0 = pl.multiple_of(i * TB, TB)
        g_s[pl.ds(r0, TB), :] = gate_act(
            _dot_nt(x_s[pl.ds(r0, TB), :], wgt_s[...]))
        return c

    jax.lax.fori_loop(NT0, NB0, gate_body, 0)
    cp_wu.wait()
    cp_wd.wait()

    def ffn_body(i, c):
        start_when(i == 0, cp_w[NB0 - 1])
        start_when(i == 1, [cp_wo])
        start_when(i == 2, [cp_x2])
        w0 = pl.multiple_of(i * WC, WC)
        pltpu.make_async_copy(wraw_s.at[pl.ds(w0, WC)],
                              wraw_s.at[pl.ds(w0, WC)], wsems.at[i]).wait()
        r0 = pl.multiple_of(i * TB, TB)
        xb = x_s[pl.ds(r0, TB), :]

        DP = 8
        todo = list(range(WC // DP))

        def relayout_piece(k):
            df = w0 + k * DP
            wi = (df >= D).astype(jnp.int32) + (df >= 2 * D).astype(jnp.int32)
            base = wi * (H * PH - D // 2) + df // 2
            uu = pltpu.bitcast(wraw_s[pl.ds(df, DP)], U32)
            t = None
            for r in range(DP // 2):
                a = uu[2 * r]
                b = uu[2 * r + 1]
                lo = (a & U32(0xFFFF)) | (b << 16)
                hi = (a >> 16) | (b & U32(0xFFFF0000))
                wqkv_s[pl.ds(base + r, H // 2, stride=2 * PH), :] = lo
                wqkv_s[pl.ds(base + PH + r, H // 2, stride=2 * PH), :] = hi
                t = (lo | hi) if t is None else (t | lo | hi)
            t = pltpu.bitcast(t[0:8] | t[8:16], jnp.int32)
            return pltpu.bitcast(jnp.minimum(t & 1, 0), U32)

        def anchor_at(m, ra, ca):
            if not todo:
                return m
            z = relayout_piece(todo.pop(0))
            blk = pltpu.bitcast(
                pltpu.bitcast(m[ra:ra + 16, ca:ca + 128], U32) | z, BF16)
            cols = [m[ra:ra + 16, :ca], blk, m[ra:ra + 16, ca + 128:]]
            mid = jnp.concatenate([q for q in cols if q.shape[1]], axis=1)
            rows = [m[:ra], mid, m[ra + 16:]]
            return jnp.concatenate([q for q in rows if q.shape[0]], axis=0)

        def anchored(m):
            for ra, ca in ANCH:
                m = anchor_at(m, ra, ca)
            return m

        hs = []
        for n in range(NC):
            c1 = min((n + 1) * CW, DFT)
            uu = _dot_nt(anchored(xb), wut_s[n * CW:c1, :])
            hs.append((g_s[pl.ds(r0, TB), n * CW:c1] * uu).astype(BF16))
        hs.append(g_s[pl.ds(r0, TB), DFT:DFP].astype(BF16))
        h = jnp.concatenate(hs, axis=1)
        for n in range(D // 128):
            bb_s[pl.ds(r0, TB), n * 128:(n + 1) * 128] = _dot(
                anchored(h), wd_s[:, n * 128:(n + 1) * 128])
        assert not todo
        return c

    jax.lax.fori_loop(0, NB0, ffn_body, 0)

    cp_wo.wait()
    cp_x2.wait()

    ri = jax.lax.broadcasted_iota(jnp.int32, (2 * L, 2 * L), 0)
    ci = jax.lax.broadcasted_iota(jnp.int32, (2 * L, 2 * L), 1)
    rhi = ri >= L
    chi = ci >= L
    rr = jnp.where(rhi, ri - L, ri)
    cc = jnp.where(chi, ci - L, ci)
    mask = (rhi == chi) & ((rr < M) | (rr >= cc))
    fill = jnp.where(rhi == chi, -1000000000.0, -jnp.inf).astype(F32)

    def w_qkv(wi, h):
        r = (wi * H + h) * PH
        return pltpu.bitcast(wqkv_s[r:r + D // 2, :], BF16)

    def softmax_pv(s, v2):
        s = jnp.where(mask, s * scale, fill)
        m = jnp.max(s, axis=-1, keepdims=True)
        p = jnp.exp(s - m)
        l = jnp.sum(p, axis=-1, keepdims=True)
        r = pl.reciprocal(l, approx=True)
        r = r * (2.0 - l * r)
        return _dot((p * r).astype(BF16), v2)

    def wo_part(rows, p0, p1):
        lhs = pltpu.bitcast(oa_s[0:rows // 2, p0 * 2 * E:p1 * 2 * E], BF16)
        rhs = wor_s[p0 * 2 * E:p1 * 2 * E, :]
        return _dot(lhs, rhs)

    def substep(hmat, is_a, sched, fillers):
        qkv = {}
        sc = {}

        def do_qkv(t):
            r = []
            for wi in range(3):
                y0 = _dot(hmat, w_qkv(wi, 2 * t))
                y1 = _dot(hmat, w_qkv(wi, 2 * t + 1))
                if is_a:
                    stq_s[wi, 2 * t] = y0[L:L + M]
                    stq_s[wi, 2 * t + 1] = y1[L:L + M]
                    z = jnp.concatenate([y0[0:L], y1[0:L]], axis=0)
                else:
                    z = jnp.concatenate(
                        [y0[0:M], stq_s[wi, 2 * t], y0[M:SEG],
                         y1[0:M], stq_s[wi, 2 * t + 1], y1[M:SEG]], axis=0)
                r.append(z.astype(BF16))
            qkv[t] = r

        def do_s(t):
            sc[t] = _dot_nt(qkv[t][0], qkv[t][1])

        def do_pv(t):
            o = softmax_pv(sc.pop(t), qkv.pop(t)[2])
            for k in range(2):
                h = 2 * t + k
                ok = o[k * L:(k + 1) * L]
                if is_a:
                    sto_s[h] = ok[SEG:L]
                    ob = ok[0:SEG].astype(BF16)
                    oa_s[0:SEG // 2, h * E:(h + 1) * E] = pltpu.bitcast(ob, U32)
                else:
                    ob = jnp.concatenate([ok, sto_s[h]], axis=0).astype(BF16)
                    oa_s[:, h * E:(h + 1) * E] = pltpu.bitcast(ob, U32)

        rows = SEG if is_a else SEG + 2 * M
        acc = None
        for op in sched:
            kind = op[0]
            if kind == 'q':
                do_qkv(op[1])
            elif kind == 's':
                do_s(op[1])
            elif kind == 'p':
                do_pv(op[1])
            elif kind == 'w':
                part = wo_part(rows, op[1], op[2])
                acc = part if acc is None else acc + part
            else:
                fillers[kind](op[1])
        return acc

    NU = len(SCHED) // 2
    RB = NU * 2 * SEG
    n_it = S // RB
    FC = DFP // 2
    FR = 2 * (S - S0) // n_it

    def seg_body(j, c):
        r0 = pl.multiple_of(j * RB, RB)
        fr0 = pl.multiple_of(S0 + (j // 2) * FR, 32)
        fc0 = pl.multiple_of((j % 2) * FC, 128)
        hs = []
        gs = {}

        def gate(k):
            xg = x_s[pl.ds(fr0, FR), :]
            c0 = pl.multiple_of(fc0 + k * 128, 128)
            gs[k] = _dot_nt(xg, wgt_s[pl.ds(c0, 128), :])

        def up(k):
            xg = x_s[pl.ds(fr0, FR), :]
            c0 = pl.multiple_of(fc0 + k * 128, 128)
            u = _dot_nt(xg, wut_s[pl.ds(c0, 128), :])
            hs.append((gelu(gs.pop(k)) * u).astype(BF16))

        def down(n):
            assert len(hs) == FC // 128
            hcat = jnp.concatenate(hs, axis=1)
            w = wd_s[pl.ds(fc0, FC), n * 128:(n + 1) * 128]
            bb_s[pl.ds(fr0, FR), n * 128:(n + 1) * 128] += _dot(hcat, w)

        def combine(iu):
            ru = pl.multiple_of(r0 + iu * 2 * SEG, 2 * SEG)
            xf = x_s[pl.ds(ru, 2 * SEG), :].astype(F32)
            z = jnp.sum(xf * gw_ref[...].astype(F32).reshape(1, D), axis=-1,
                        keepdims=True)
            gt = jax.nn.sigmoid(z)
            out_s[pl.ds(ru, 2 * SEG), :] = (
                gt * outs.pop(iu) + (1.0 - gt) * bb_s[pl.ds(ru, 2 * SEG), :]
            ).astype(out_s.dtype)

        outs = {}
        fills = dict(g=gate, u=up, d=down, c=combine)

        mem = mem_s[...]
        for iu in range(NU):
            ru = pl.multiple_of(r0 + iu * 2 * SEG, 2 * SEG)
            xf = x_s[pl.ds(ru, 2 * SEG), :].astype(F32)
            ha = jnp.concatenate([mem, xf[0:L]], axis=0).astype(BF16)
            acc_a = substep(ha, True, SCHED[2 * iu], fills)
            hb = jnp.concatenate([acc_a[0:M], xf[L:2 * SEG]],
                                 axis=0).astype(BF16)
            acc_b = substep(hb, False, SCHED[2 * iu + 1], fills)
            mem = acc_b[0:M]
            outs[iu] = jnp.concatenate(
                [acc_a[M:SEG], acc_b[L:L + M], acc_b[M:L]], axis=0)
        mem_s[...] = mem
        for iu in list(outs):
            combine(iu)
        pltpu.make_async_copy(out_s.at[pl.ds(r0, RB)],
                              out_hbm.at[pl.ds(r0, RB)], osem).start()
        return c

    jax.lax.fori_loop(0, n_it, seg_body, 0)
    pltpu.make_async_copy(out_s, out_hbm, osem).wait()


@jax.jit
def pallas_gated_mix__memory_aug_recurrent_mem_tr__glu_gated_geglu__prompt_kernel(
    A_x: jax.Array,
    A_mem0: jax.Array,
    A_Wq: jax.Array,
    A_Wk: jax.Array,
    A_Wv: jax.Array,
    A_Wo: jax.Array,
    A_seg_len: jax.Array,
    B_x: jax.Array,
    B_w_gate: jax.Array,
    B_w_up: jax.Array,
    B_w_down: jax.Array,
    gate_w: jax.Array,
):
    B, S, D = A_x.shape
    H, E = A_Wq.shape[1], A_Wq.shape[2]
    M = A_mem0.shape[1]
    DF = B_w_gate.shape[1]
    DFP = -(-DF // 256) * 256
    SEG = 32
    assert B == 1 and M == 8 and S == 2048 and D == 640 and H == 32

    kern = functools.partial(_kernel, S=S, D=D, H=H, E=E, M=M, SEG=SEG, DF=DF,
                             DFP=DFP)
    hbm = pl.BlockSpec(memory_space=pl.ANY)
    vm = pl.BlockSpec(memory_space=pltpu.VMEM)
    out = pl.pallas_call(
        kern,
        out_shape=jax.ShapeDtypeStruct((S, D), A_x.dtype),
        in_specs=[hbm, vm, hbm, hbm, hbm, hbm, hbm, hbm, hbm, vm],
        out_specs=hbm,
        scratch_shapes=[
            pltpu.VMEM((S, D), BF16),
            pltpu.VMEM((3 * D, H, E), BF16),
            pltpu.VMEM((H * E, D), BF16),
            pltpu.VMEM((DFP, D), BF16),
            pltpu.VMEM((DFP, D), BF16),
            pltpu.VMEM((DFP, D), BF16),
            pltpu.VMEM((3 * H * PH_, E), U32),
            pltpu.VMEM((S, D), F32),
            pltpu.VMEM((5 * 256, DFP), F32),
            pltpu.VMEM((M, D), F32),
            pltpu.VMEM((3, H, M, E), F32),
            pltpu.VMEM((H, M, E), F32),
            pltpu.VMEM(((SEG + 2 * M) // 2, H * E), U32),
            pltpu.VMEM((S, D), BF16),
            pltpu.SemaphoreType.DMA((10,)),
            pltpu.SemaphoreType.DMA((5,)),
            pltpu.SemaphoreType.DMA,
        ],
        compiler_params=pltpu.CompilerParams(
            vmem_limit_bytes=110 * 1024 * 1024),
    )(
        A_x.reshape(S, D), A_mem0.reshape(M, D), A_Wq, A_Wk, A_Wv,
        A_Wo.reshape(H * E, D), B_w_gate.T, B_w_up.T, B_w_down,
        gate_w,
    )
    return out.reshape(B, S, D)
```

```python
import functools

import jax
import jax.numpy as jnp
import jax.experimental.pallas as pl
import jax.experimental.pallas.tpu as pltpu

F32 = jnp.float32
BF16 = jnp.bfloat16
U32 = jnp.uint32
PH_ = 321
ANCH = ((64, 0), (192, 128), (64, 384), (192, 512))
ANCHD = ANCH


def _mk_sched(cfg):
    NP = 16
    dp, ds = cfg.get('dp', 3), cfg.get('ds', 1)
    fill = {}
    for pos, f in cfg.get('fill', []):
        fill.setdefault(str(pos), []).append(tuple(f))
    early = {int(k): v for k, v in cfg.get('early_w', {}).items()}
    out = list(fill.get('start', []))
    for t in range(NP):
        out.append(('q', t))
        if t >= dp:
            out.append(('p', t - dp))
        if t >= ds:
            out.append(('s', t - ds))
        if t in early:
            out.append(('w',) + tuple(early[t]))
        out += fill.get(str(t), [])
    for k, op in enumerate(cfg['tail']):
        out.append(tuple(op))
        out += fill.get('t%d' % k, [])
    return out


_T = dict(
    T1=dict(early_w={'14': [0, 2]},
            tail=[['w', 2, 5], ['p', 13], ['s', 15], ['w', 5, 8], ['p', 14],
                  ['w', 8, 12], ['p', 15], ['w', 12, 15], ['w', 15, 16]]),
    T3=dict(early_w={'13': [0, 1], '14': [1, 2]},
            tail=[['w', 2, 5], ['p', 13], ['s', 15], ['w', 5, 8], ['p', 14],
                  ['w', 8, 12], ['p', 15], ['w', 12, 15], ['w', 15, 16]]),
    T6=dict(early_w={'12': [0, 2], '14': [2, 4]},
            tail=[['w', 4, 6], ['p', 13], ['s', 15], ['w', 6, 9], ['p', 14],
                  ['w', 9, 12], ['p', 15], ['w', 12, 15], ['w', 15, 16]]),
)
_CFG = [
    ['T1', [[4, ['g', 0]], [8, ['u', 0]], ['t7', ['g', 1]], ['t8', ['u', 1]]]],
    ['T1', [[2, ['g', 2]], [5, ['u', 2]], [8, ['g', 3]], [11, ['u', 3]],
            ['t7', ['g', 4]], ['t8', ['u', 4]]]],
    ['T1', [[2, ['g', 5]], [4, ['u', 5]], [6, ['g', 6]], [8, ['u', 6]],
            ['t7', ['d', 0]], ['t8', ['d', 1]]]],
    ['T1', [[2, ['d', 2]], [5, ['d', 3]], [8, ['d', 4]], [10, ['c', 0]]]],
]
SCHED = [_mk_sched(dict(_T[t], fill=f)) for t, f in _CFG]


def _dot(a, b):
    return jnp.dot(a, b, preferred_element_type=F32)


def _dot_nt(a, b):
    return jax.lax.dot_general(a, b, (((1,), (1,)), ((), ())),
                               preferred_element_type=F32)


def _kernel(x_hbm, mem0_ref, wq_hbm, wk_hbm, wv_hbm, wo_hbm, wgt_hbm, wut_hbm,
            wd_hbm, gw_ref, out_hbm,
            x_s, wraw_s, wor_s, wgt_s, wut_s, wd_s, wqkv_s, bb_s, g_s,
            mem_s, stq_s, sto_s, oa_s, out_s, sems, wsems, osem,
            *, S, D, H, E, M, SEG, DF, DFP):
    L = M + SEG
    PH = PH_
    scale = float(E) ** -0.5
    TB = 256
    NB0 = 5
    S0 = NB0 * TB
    CW = 256
    NC = DFP // CW
    DFT = DFP - 128
    assert DFP - DF == DF - DFT == 64
    WC = 3 * D // NB0

    GCH = (0, 256, 768, DF)

    def xcopy(a, b, k):
        return pltpu.make_async_copy(x_hbm.at[pl.ds(a, b - a)],
                                     x_s.at[pl.ds(a, b - a)], sems.at[k])

    NT0 = 2
    T0 = NT0 * TB
    STG = 1
    cp_x0 = xcopy(0, T0, 0)
    cp_wg = [pltpu.make_async_copy(
        wgt_hbm.at[pl.ds(GCH[k], GCH[k + 1] - GCH[k])],
        wgt_s.at[pl.ds(GCH[k], GCH[k + 1] - GCH[k])], sems.at[1 + k])
        for k in range(3)]
    cp_wm = pltpu.make_async_copy(wut_hbm.at[pl.ds(DFT, DF - DFT)],
                                  wgt_s.at[pl.ds(DF, DFP - DF)], sems.at[4])
    cp_x1 = xcopy(T0, S0, 5)
    cp_wu = pltpu.make_async_copy(wut_hbm, wut_s.at[pl.ds(0, DF)], sems.at[6])
    cp_wd = pltpu.make_async_copy(wd_hbm, wd_s.at[pl.ds(0, DF)], sems.at[7])
    cp_w = []
    for c in range(NB0):
        a = c * WC
        cp_w.append([])
        while a < (c + 1) * WC:
            wi = a // D
            b = min((c + 1) * WC, (wi + 1) * D)
            cp_w[c].append(pltpu.make_async_copy(
                (wq_hbm, wk_hbm, wv_hbm)[wi].at[pl.ds(a - wi * D, b - a)],
                wraw_s.at[pl.ds(a, b - a)], wsems.at[c]))
            a = b

    def start_when(cond, cps):
        @pl.when(cond)
        def _():
            for cp in cps:
                cp.start()
    cp_wo = pltpu.make_async_copy(wo_hbm, wor_s, sems.at[8])
    cp_x2 = xcopy(S0, S, 9)
    cp_x0.start()
    cp_wg[0].start()
    if STG == 0:
        cp_wg[1].start()
        cp_wg[2].start()
        cp_wm.start()
        cp_x1.start()
    if STG == 1:
        cp_wg[1].start()

    zpad = jnp.zeros((DFP - DF, D), BF16)
    wut_s[DF:DFP, :] = zpad
    wd_s[DF:DFP, :] = zpad
    bb_s[S0:S, :] = jnp.zeros((S - S0, D), F32)
    mem_s[...] = mem0_ref[...].astype(F32)

    def gelu(g):
        return jax.nn.gelu(g, approximate=True)

    def gate_store(xb, rows, c0):
        t = _dot_nt(xb, wgt_s[DFT:DFP, :])
        lane = jax.lax.broadcasted_iota(jnp.int32, t.shape, 1)
        g_s[rows, DFT:DFP] = jnp.where(
            lane < 64, gelu(t) * pltpu.roll(t, 64, 1), 0.0)
        g_s[rows, c0:DFT] = gelu(_dot_nt(xb, wgt_s[c0:DFT, :]))

    if STG == 2:
        cp_wg[1].start()
    cp_x0.wait()
    cp_wg[0].wait()
    if STG == 0:
        cp_wu.start()
        cp_wd.start()
    else:
        cp_wg[2].start()
        cp_wm.start()
        cp_x1.start()
    xb = x_s[0:T0, :]
    g_s[0:T0, GCH[0]:GCH[1]] = gelu(_dot_nt(xb, wgt_s[GCH[0]:GCH[1], :]))
    cp_wg[1].wait()
    if STG:
        cp_wu.start()
    g_s[0:T0, GCH[1]:GCH[2]] = gelu(_dot_nt(xb, wgt_s[GCH[1]:GCH[2], :]))
    cp_wg[2].wait()
    cp_wm.wait()
    if STG:
        cp_wd.start()
    if NT0 == 2:
        for cp in cp_w[0]:
            cp.start()
    gate_store(xb, pl.ds(0, T0), GCH[2])
    cp_x1.wait()

    def gate_body(i, c):
        for k in range(NT0, NB0):
            start_when(i == k, cp_w[k - 1])
        r0 = pl.multiple_of(i * TB, TB)
        gate_store(x_s[pl.ds(r0, TB), :], pl.ds(r0, TB), 0)
        return c

    jax.lax.fori_loop(NT0, NB0, gate_body, 0)
    cp_wu.wait()
    cp_wd.wait()

    def ffn_body(i, c):
        start_when(i == 0, cp_w[NB0 - 1])
        start_when(i == 1, [cp_wo])
        start_when(i == 2, [cp_x2])
        w0 = pl.multiple_of(i * WC, WC)
        pltpu.make_async_copy(wraw_s.at[pl.ds(w0, WC)],
                              wraw_s.at[pl.ds(w0, WC)], wsems.at[i]).wait()
        r0 = pl.multiple_of(i * TB, TB)
        xb = x_s[pl.ds(r0, TB), :]

        DP = 8
        todo = list(range(WC // DP))

        def relayout_piece(k):
            df = w0 + k * DP
            wi = (df >= D).astype(jnp.int32) + (df >= 2 * D).astype(jnp.int32)
            base = wi * (H * PH - D // 2) + df // 2
            uu = pltpu.bitcast(wraw_s[pl.ds(df, DP)], U32)
            t = None
            for r in range(DP // 2):
                a = uu[2 * r]
                b = uu[2 * r + 1]
                lo = (a & U32(0xFFFF)) | (b << 16)
                hi = (a >> 16) | (b & U32(0xFFFF0000))
                wqkv_s[pl.ds(base + r, H // 2, stride=2 * PH), :] = lo
                wqkv_s[pl.ds(base + PH + r, H // 2, stride=2 * PH), :] = hi
                t = (lo | hi) if t is None else (t | lo | hi)
            t = pltpu.bitcast(t[0:8] | t[8:16], jnp.int32)
            return pltpu.bitcast(jnp.minimum(t & 1, 0), U32)

        def anchor_at(m, ra, ca):
            if not todo:
                return m
            z = relayout_piece(todo.pop(0))
            blk = pltpu.bitcast(
                pltpu.bitcast(m[ra:ra + 16, ca:ca + 128], U32) | z, BF16)
            cols = [m[ra:ra + 16, :ca], blk, m[ra:ra + 16, ca + 128:]]
            mid = jnp.concatenate([q for q in cols if q.shape[1]], axis=1)
            rows = [m[:ra], mid, m[ra + 16:]]
            return jnp.concatenate([q for q in rows if q.shape[0]], axis=0)

        def anchored(m, pos=ANCH):
            for ra, ca in pos:
                m = anchor_at(m, ra, ca)
            return m

        hs = []
        for n in range(NC):
            c1 = min((n + 1) * CW, DFT)
            uu = _dot_nt(anchored(xb), wut_s[n * CW:c1, :])
            hs.append((g_s[pl.ds(r0, TB), n * CW:c1] * uu).astype(BF16))
        hs.append(g_s[pl.ds(r0, TB), DFT:DFP].astype(BF16))
        h = jnp.concatenate(hs, axis=1)
        for n in range(D // 128):
            bb_s[pl.ds(r0, TB), n * 128:(n + 1) * 128] = _dot(
                anchored(h, ANCHD), wd_s[:, n * 128:(n + 1) * 128])
        assert not todo
        return c

    jax.lax.fori_loop(0, NB0, ffn_body, 0)

    cp_wo.wait()
    cp_x2.wait()

    ri = jax.lax.broadcasted_iota(jnp.int32, (2 * L, 2 * L), 0)
    ci = jax.lax.broadcasted_iota(jnp.int32, (2 * L, 2 * L), 1)
    rhi = ri >= L
    chi = ci >= L
    rr = jnp.where(rhi, ri - L, ri)
    cc = jnp.where(chi, ci - L, ci)
    mask = (rhi == chi) & ((rr < M) | (rr >= cc))
    fill = jnp.where(rhi == chi, -1000000000.0, -jnp.inf).astype(F32)

    def w_qkv(wi, h):
        r = (wi * H + h) * PH
        return pltpu.bitcast(wqkv_s[r:r + D // 2, :], BF16)

    def softmax_pv(s, v2):
        s = jnp.where(mask, s * scale, fill)
        m = jnp.max(s, axis=-1, keepdims=True)
        p = jnp.exp(s - m)
        l = jnp.sum(p, axis=-1, keepdims=True)
        r = pl.reciprocal(l, approx=True)
        r = r * (2.0 - l * r)
        return _dot((p * r).astype(BF16), v2)

    def wo_part(rows, p0, p1):
        lhs = pltpu.bitcast(oa_s[0:rows // 2, p0 * 2 * E:p1 * 2 * E], BF16)
        rhs = wor_s[p0 * 2 * E:p1 * 2 * E, :]
        return _dot(lhs, rhs)

    def substep(hmat, is_a, sched, fillers):
        qkv = {}
        sc = {}

        def do_qkv(t):
            r = []
            for wi in range(3):
                y0 = _dot(hmat, w_qkv(wi, 2 * t))
                y1 = _dot(hmat, w_qkv(wi, 2 * t + 1))
                if is_a:
                    stq_s[wi, 2 * t] = y0[L:L + M]
                    stq_s[wi, 2 * t + 1] = y1[L:L + M]
                    z = jnp.concatenate([y0[0:L], y1[0:L]], axis=0)
                else:
                    z = jnp.concatenate(
                        [y0[0:M], stq_s[wi, 2 * t], y0[M:SEG],
                         y1[0:M], stq_s[wi, 2 * t + 1], y1[M:SEG]], axis=0)
                r.append(z.astype(BF16))
            qkv[t] = r

        def do_s(t):
            sc[t] = _dot_nt(qkv[t][0], qkv[t][1])

        def do_pv(t):
            o = softmax_pv(sc.pop(t), qkv.pop(t)[2])
            for k in range(2):
                h = 2 * t + k
                ok = o[k * L:(k + 1) * L]
                if is_a:
                    sto_s[h] = ok[SEG:L]
                    ob = ok[0:SEG].astype(BF16)
                    oa_s[0:SEG // 2, h * E:(h + 1) * E] = pltpu.bitcast(ob, U32)
                else:
                    ob = jnp.concatenate([ok, sto_s[h]], axis=0).astype(BF16)
                    oa_s[:, h * E:(h + 1) * E] = pltpu.bitcast(ob, U32)

        rows = SEG if is_a else SEG + 2 * M
        acc = None
        for op in sched:
            kind = op[0]
            if kind == 'q':
                do_qkv(op[1])
            elif kind == 's':
                do_s(op[1])
            elif kind == 'p':
                do_pv(op[1])
            elif kind == 'w':
                part = wo_part(rows, op[1], op[2])
                acc = part if acc is None else acc + part
            else:
                fillers[kind](op[1])
        return acc

    NU = len(SCHED) // 2
    RB = NU * 2 * SEG
    n_it = S // RB
    FC = DFP // 2
    FR = 2 * (S - S0) // n_it

    def seg_body(j, c):
        r0 = pl.multiple_of(j * RB, RB)
        fr0 = pl.multiple_of(S0 + (j // 2) * FR, 32)
        fc0 = pl.multiple_of((j % 2) * FC, 128)
        hs = []
        gs = {}

        def gate(k):
            xg = x_s[pl.ds(fr0, FR), :]
            c0 = pl.multiple_of(fc0 + k * 128, 128)
            gs[k] = _dot_nt(xg, wgt_s[pl.ds(c0, 128), :])

        def up(k):
            xg = x_s[pl.ds(fr0, FR), :]
            c0 = pl.multiple_of(fc0 + k * 128, 128)
            u = _dot_nt(xg, wut_s[pl.ds(c0, 128), :])
            hs.append((gelu(gs.pop(k)) * u).astype(BF16))

        def down(n):
            assert len(hs) == FC // 128
            hcat = jnp.concatenate(hs, axis=1)
            w = wd_s[pl.ds(fc0, FC), n * 128:(n + 1) * 128]
            bb_s[pl.ds(fr0, FR), n * 128:(n + 1) * 128] += _dot(hcat, w)

        def combine(iu):
            ru = pl.multiple_of(r0 + iu * 2 * SEG, 2 * SEG)
            xf = x_s[pl.ds(ru, 2 * SEG), :].astype(F32)
            z = jnp.sum(xf * gw_ref[...].astype(F32).reshape(1, D), axis=-1,
                        keepdims=True)
            gt = jax.nn.sigmoid(z)
            out_s[pl.ds(ru, 2 * SEG), :] = (
                gt * outs.pop(iu) + (1.0 - gt) * bb_s[pl.ds(ru, 2 * SEG), :]
            ).astype(out_s.dtype)

        outs = {}
        fills = dict(g=gate, u=up, d=down, c=combine)

        mem = mem_s[...]
        for iu in range(NU):
            ru = pl.multiple_of(r0 + iu * 2 * SEG, 2 * SEG)
            xf = x_s[pl.ds(ru, 2 * SEG), :].astype(F32)
            ha = jnp.concatenate([mem, xf[0:L]], axis=0).astype(BF16)
            acc_a = substep(ha, True, SCHED[2 * iu], fills)
            hb = jnp.concatenate([acc_a[0:M], xf[L:2 * SEG]],
                                 axis=0).astype(BF16)
            acc_b = substep(hb, False, SCHED[2 * iu + 1], fills)
            mem = acc_b[0:M]
            outs[iu] = jnp.concatenate(
                [acc_a[M:SEG], acc_b[L:L + M], acc_b[M:L]], axis=0)
        mem_s[...] = mem
        for iu in list(outs):
            combine(iu)
        pltpu.make_async_copy(out_s.at[pl.ds(r0, RB)],
                              out_hbm.at[pl.ds(r0, RB)], osem).start()
        return c

    jax.lax.fori_loop(0, n_it, seg_body, 0)
    pltpu.make_async_copy(out_s, out_hbm, osem).wait()


@jax.jit
def pallas_gated_mix__memory_aug_recurrent_mem_tr__glu_gated_geglu__prompt_kernel(
    A_x: jax.Array,
    A_mem0: jax.Array,
    A_Wq: jax.Array,
    A_Wk: jax.Array,
    A_Wv: jax.Array,
    A_Wo: jax.Array,
    A_seg_len: jax.Array,
    B_x: jax.Array,
    B_w_gate: jax.Array,
    B_w_up: jax.Array,
    B_w_down: jax.Array,
    gate_w: jax.Array,
):
    B, S, D = A_x.shape
    H, E = A_Wq.shape[1], A_Wq.shape[2]
    M = A_mem0.shape[1]
    DF = B_w_gate.shape[1]
    DFP = -(-DF // 256) * 256
    SEG = 32
    assert B == 1 and M == 8 and S == 2048 and D == 640 and H == 32

    kern = functools.partial(_kernel, S=S, D=D, H=H, E=E, M=M, SEG=SEG, DF=DF,
                             DFP=DFP)
    hbm = pl.BlockSpec(memory_space=pl.ANY)
    vm = pl.BlockSpec(memory_space=pltpu.VMEM)
    out = pl.pallas_call(
        kern,
        out_shape=jax.ShapeDtypeStruct((S, D), A_x.dtype),
        in_specs=[hbm, vm, hbm, hbm, hbm, hbm, hbm, hbm, hbm, vm],
        out_specs=hbm,
        scratch_shapes=[
            pltpu.VMEM((S, D), BF16),
            pltpu.VMEM((3 * D, H, E), BF16),
            pltpu.VMEM((H * E, D), BF16),
            pltpu.VMEM((DFP, D), BF16),
            pltpu.VMEM((DFP, D), BF16),
            pltpu.VMEM((DFP, D), BF16),
            pltpu.VMEM(((3 * H + 3) * PH_ + 5, E), U32),
            pltpu.VMEM((S, D), F32),
            pltpu.VMEM((5 * 256, DFP), F32),
            pltpu.VMEM((M, D), F32),
            pltpu.VMEM((3, H, M, E), F32),
            pltpu.VMEM((H, M, E), F32),
            pltpu.VMEM(((SEG + 2 * M) // 2, H * E), U32),
            pltpu.VMEM((S, D), BF16),
            pltpu.SemaphoreType.DMA((10,)),
            pltpu.SemaphoreType.DMA((5,)),
            pltpu.SemaphoreType.DMA,
        ],
        compiler_params=pltpu.CompilerParams(
            vmem_limit_bytes=110 * 1024 * 1024),
    )(
        A_x.reshape(S, D), A_mem0.reshape(M, D), A_Wq, A_Wk, A_Wv,
        A_Wo.reshape(H * E, D), B_w_gate.T, B_w_up.T, B_w_down,
        gate_w,
    )
    return out.reshape(B, S, D)
```

```python
import functools

import jax
import jax.numpy as jnp
import jax.experimental.pallas as pl
import jax.experimental.pallas.tpu as pltpu

F32 = jnp.float32
BF16 = jnp.bfloat16
U32 = jnp.uint32
PH_ = 321
ANCH = ((64, 0), (192, 128), (64, 384), (192, 512))
ANCHD = ANCH


def _mk_sched(cfg):
    NP = 16
    dp, ds = cfg.get('dp', 3), cfg.get('ds', 1)
    fill = {}
    for pos, f in cfg.get('fill', []):
        fill.setdefault(str(pos), []).append(tuple(f))
    early = {int(k): v for k, v in cfg.get('early_w', {}).items()}
    out = list(fill.get('start', []))
    for t in range(NP):
        out.append(('q', t))
        if t >= dp:
            out.append(('p', t - dp))
        if t >= ds:
            out.append(('s', t - ds))
        if t in early:
            out.append(('w',) + tuple(early[t]))
        out += fill.get(str(t), [])
    for k, op in enumerate(cfg['tail']):
        out.append(tuple(op))
        out += fill.get('t%d' % k, [])
    return out


_T = dict(
    T1=dict(early_w={'14': [0, 2]},
            tail=[['w', 2, 5], ['p', 13], ['s', 15], ['w', 5, 8], ['p', 14],
                  ['w', 8, 12], ['p', 15], ['w', 12, 15], ['w', 15, 16]]),
)
_CFG = [
    ['T1', [[4, ['g', 0]], [8, ['u', 0]], ['t7', ['g', 1]], ['t8', ['u', 1]]]],
    ['T1', [[2, ['g', 2]], [5, ['u', 2]], [8, ['g', 3]], [11, ['u', 3]],
            ['t7', ['g', 4]], ['t8', ['u', 4]]]],
    ['T1', [[2, ['g', 5]], [4, ['u', 5]], [6, ['g', 6]], [8, ['u', 6]],
            ['t7', ['d', 0]], ['t8', ['d', 1]]]],
    ['T1', [[2, ['d', 2]], [5, ['d', 3]], [8, ['d', 4]], [10, ['c', 0]]]],
]
SCHED = [_mk_sched(dict(_T[t], fill=f)) for t, f in _CFG]


def _dot(a, b):
    return jnp.dot(a, b, preferred_element_type=F32)


def _dot_nt(a, b):
    return jax.lax.dot_general(a, b, (((1,), (1,)), ((), ())),
                               preferred_element_type=F32)


def _kernel(x_hbm, mem0_hbm, wq_hbm, wk_hbm, wv_hbm, wo_hbm, wgt_hbm, wut_hbm,
            wd_hbm, gw_hbm, out_hbm,
            x_s, wraw_s, wor_s, wgt_s, wut_s, wd_s, wqkv_s, bb_s, g_s,
            mem_s, stq_s, sto_s, oa_s, out_s, mem0_ref, gw_ref,
            sems, wsems, osem,
            *, S, D, H, E, M, SEG, DF, DFP):
    L = M + SEG
    PH = PH_
    scale = float(E) ** -0.5
    TB = 256
    NB0 = 5
    S0 = NB0 * TB
    CW = 256
    NC = DFP // CW
    DFT = DFP - 128
    assert DFP - DF == DF - DFT == 64
    WC = 3 * D // NB0

    GCH = (0, 256, 768, DF)

    def xcopy(a, b, k):
        return pltpu.make_async_copy(x_hbm.at[pl.ds(a, b - a)],
                                     x_s.at[pl.ds(a, b - a)], sems.at[k])

    NT0 = 2
    T0 = NT0 * TB
    cp_x0 = xcopy(0, T0, 0)
    cp_wg = [pltpu.make_async_copy(
        wgt_hbm.at[pl.ds(GCH[k], GCH[k + 1] - GCH[k])],
        wgt_s.at[pl.ds(GCH[k], GCH[k + 1] - GCH[k])], sems.at[1 + k])
        for k in range(3)]
    cp_wm = pltpu.make_async_copy(wut_hbm.at[pl.ds(DFT, DF - DFT)],
                                  wgt_s.at[pl.ds(DF, DFP - DF)], sems.at[4])
    cp_x1 = xcopy(T0, S0, 5)
    cp_wu = pltpu.make_async_copy(wut_hbm, wut_s.at[pl.ds(0, DF)], sems.at[6])
    cp_wd = pltpu.make_async_copy(wd_hbm, wd_s.at[pl.ds(0, DF)], sems.at[7])
    cp_w = []
    for c in range(NB0):
        a = c * WC
        cp_w.append([])
        while a < (c + 1) * WC:
            wi = a // D
            b = min((c + 1) * WC, (wi + 1) * D)
            cp_w[c].append(pltpu.make_async_copy(
                (wq_hbm, wk_hbm, wv_hbm)[wi].at[pl.ds(a - wi * D, b - a)],
                wraw_s.at[pl.ds(a, b - a)], wsems.at[c]))
            a = b

    def start_when(cond, cps):
        @pl.when(cond)
        def _():
            for cp in cps:
                cp.start()

    cp_wo = pltpu.make_async_copy(wo_hbm, wor_s, sems.at[8])
    cp_x2 = xcopy(S0, S, 9)
    cp_m0 = pltpu.make_async_copy(mem0_hbm, mem0_ref, sems.at[10])
    cp_gw = pltpu.make_async_copy(gw_hbm, gw_ref, sems.at[11])
    cp_x0.start()
    cp_wg[0].start()
    cp_wg[1].start()

    zpad = jnp.zeros((DFP - DF, D), BF16)
    wut_s[DF:DFP, :] = zpad
    wd_s[DF:DFP, :] = zpad
    bb_s[S0:S, :] = jnp.zeros((S - S0, D), F32)

    def gelu(g):
        return jax.nn.gelu(g, approximate=True)

    def gate_store(xb, rows, c0):
        t = _dot_nt(xb, wgt_s[DFT:DFP, :])
        lane = jax.lax.broadcasted_iota(jnp.int32, t.shape, 1)
        g_s[rows, DFT:DFP] = jnp.where(
            lane < 64, gelu(t) * pltpu.roll(t, 64, 1), 0.0)
        g_s[rows, c0:DFT] = gelu(_dot_nt(xb, wgt_s[c0:DFT, :]))

    cp_x0.wait()
    cp_wg[0].wait()
    cp_wg[2].start()
    cp_wm.start()
    cp_x1.start()
    xb = x_s[0:T0, :]
    g_s[0:T0, GCH[0]:GCH[1]] = gelu(_dot_nt(xb, wgt_s[GCH[0]:GCH[1], :]))
    cp_wg[1].wait()
    cp_wu.start()
    g_s[0:T0, GCH[1]:GCH[2]] = gelu(_dot_nt(xb, wgt_s[GCH[1]:GCH[2], :]))
    cp_wg[2].wait()
    cp_wm.wait()
    cp_wd.start()
    for cp in cp_w[0]:
        cp.start()
    gate_store(xb, pl.ds(0, T0), GCH[2])
    cp_x1.wait()

    def gate_body(i, c):
        for k in range(NT0, NB0):
            start_when(i == k, cp_w[k - 1])
        r0 = pl.multiple_of(i * TB, TB)
        gate_store(x_s[pl.ds(r0, TB), :], pl.ds(r0, TB), 0)
        return c

    jax.lax.fori_loop(NT0, NB0, gate_body, 0)
    cp_wu.wait()
    cp_wd.wait()

    def ffn_body(i, c):
        start_when(i == 0, cp_w[NB0 - 1])
        start_when(i == 1, [cp_wo])
        start_when(i == 2, [cp_x2, cp_m0, cp_gw])
        w0 = pl.multiple_of(i * WC, WC)
        pltpu.make_async_copy(wraw_s.at[pl.ds(w0, WC)],
                              wraw_s.at[pl.ds(w0, WC)], wsems.at[i]).wait()
        r0 = pl.multiple_of(i * TB, TB)
        xb = x_s[pl.ds(r0, TB), :]

        DP = 8
        todo = list(range(WC // DP))

        def relayout_piece(k):
            df = w0 + k * DP
            wi = (df >= D).astype(jnp.int32) + (df >= 2 * D).astype(jnp.int32)
            base = wi * (H * PH - D // 2) + df // 2
            uu = pltpu.bitcast(wraw_s[pl.ds(df, DP)], U32)
            t = None
            for r in range(DP // 2):
                a = uu[2 * r]
                b = uu[2 * r + 1]
                lo = (a & U32(0xFFFF)) | (b << 16)
                hi = (a >> 16) | (b & U32(0xFFFF0000))
                wqkv_s[pl.ds(base + r, H // 2, stride=2 * PH), :] = lo
                wqkv_s[pl.ds(base + PH + r, H // 2, stride=2 * PH), :] = hi
                t = (lo | hi) if t is None else (t | lo | hi)
            t = pltpu.bitcast(t[0:8] | t[8:16], jnp.int32)
            return pltpu.bitcast(jnp.minimum(t & 1, 0), U32)

        def anchor_at(m, ra, ca):
            if not todo:
                return m
            z = relayout_piece(todo.pop(0))
            blk = pltpu.bitcast(
                pltpu.bitcast(m[ra:ra + 16, ca:ca + 128], U32) | z, BF16)
            cols = [m[ra:ra + 16, :ca], blk, m[ra:ra + 16, ca + 128:]]
            mid = jnp.concatenate([q for q in cols if q.shape[1]], axis=1)
            rows = [m[:ra], mid, m[ra + 16:]]
            return jnp.concatenate([q for q in rows if q.shape[0]], axis=0)

        def anchored(m, pos=ANCH):
            for ra, ca in pos:
                m = anchor_at(m, ra, ca)
            return m

        hs = []
        for n in range(NC):
            c1 = min((n + 1) * CW, DFT)
            uu = _dot_nt(anchored(xb), wut_s[n * CW:c1, :])
            hs.append((g_s[pl.ds(r0, TB), n * CW:c1] * uu).astype(BF16))
        hs.append(g_s[pl.ds(r0, TB), DFT:DFP].astype(BF16))
        h = jnp.concatenate(hs, axis=1)
        for n in range(D // 128):
            bb_s[pl.ds(r0, TB), n * 128:(n + 1) * 128] = _dot(
                anchored(h, ANCHD), wd_s[:, n * 128:(n + 1) * 128])
        assert not todo
        return c

    jax.lax.fori_loop(0, NB0, ffn_body, 0)

    cp_wo.wait()
    cp_x2.wait()
    cp_m0.wait()
    cp_gw.wait()
    mem_s[...] = mem0_ref[...].astype(F32)

    ri = jax.lax.broadcasted_iota(jnp.int32, (2 * L, 2 * L), 0)
    ci = jax.lax.broadcasted_iota(jnp.int32, (2 * L, 2 * L), 1)
    rhi = ri >= L
    chi = ci >= L
    rr = jnp.where(rhi, ri - L, ri)
    cc = jnp.where(chi, ci - L, ci)
    mask = (rhi == chi) & ((rr < M) | (rr >= cc))
    fill = jnp.where(rhi == chi, -1000000000.0, -jnp.inf).astype(F32)

    def w_qkv(wi, h):
        r = (wi * H + h) * PH
        return pltpu.bitcast(wqkv_s[r:r + D // 2, :], BF16)

    def softmax_pv(s, v2):
        s = jnp.where(mask, s * scale, fill)
        m = jnp.max(s, axis=-1, keepdims=True)
        p = jnp.exp(s - m)
        l = jnp.sum(p, axis=-1, keepdims=True)
        r = pl.reciprocal(l, approx=True)
        r = r * (2.0 - l * r)
        return _dot((p * r).astype(BF16), v2)

    def wo_part(rows, p0, p1):
        lhs = pltpu.bitcast(oa_s[0:rows // 2, p0 * 2 * E:p1 * 2 * E], BF16)
        rhs = wor_s[p0 * 2 * E:p1 * 2 * E, :]
        return _dot(lhs, rhs)

    def substep(hmat, is_a, sched, fillers):
        qkv = {}
        sc = {}

        def do_qkv(t):
            r = []
            for wi in range(3):
                y0 = _dot(hmat, w_qkv(wi, 2 * t))
                y1 = _dot(hmat, w_qkv(wi, 2 * t + 1))
                if is_a:
                    stq_s[wi, 2 * t] = y0[L:L + M]
                    stq_s[wi, 2 * t + 1] = y1[L:L + M]
                    z = jnp.concatenate([y0[0:L], y1[0:L]], axis=0)
                else:
                    z = jnp.concatenate(
                        [y0[0:M], stq_s[wi, 2 * t], y0[M:SEG],
                         y1[0:M], stq_s[wi, 2 * t + 1], y1[M:SEG]], axis=0)
                r.append(z.astype(BF16))
            qkv[t] = r

        def do_s(t):
            sc[t] = _dot_nt(qkv[t][0], qkv[t][1])

        def do_pv(t):
            o = softmax_pv(sc.pop(t), qkv.pop(t)[2])
            for k in range(2):
                h = 2 * t + k
                ok = o[k * L:(k + 1) * L]
                if is_a:
                    sto_s[h] = ok[SEG:L]
                    ob = ok[0:SEG].astype(BF16)
                    oa_s[0:SEG // 2, h * E:(h + 1) * E] = pltpu.bitcast(ob, U32)
                else:
                    ob = jnp.concatenate([ok, sto_s[h]], axis=0).astype(BF16)
                    oa_s[:, h * E:(h + 1) * E] = pltpu.bitcast(ob, U32)

        rows = SEG if is_a else SEG + 2 * M
        acc = None
        for op in sched:
            kind = op[0]
            if kind == 'q':
                do_qkv(op[1])
            elif kind == 's':
                do_s(op[1])
            elif kind == 'p':
                do_pv(op[1])
            elif kind == 'w':
                part = wo_part(rows, op[1], op[2])
                acc = part if acc is None else acc + part
            else:
                fillers[kind](op[1])
        return acc

    NU = len(SCHED) // 2
    RB = NU * 2 * SEG
    n_it = S // RB
    FC = DFP // 2
    FR = 2 * (S - S0) // n_it

    def seg_body(j, c):
        r0 = pl.multiple_of(j * RB, RB)
        fr0 = pl.multiple_of(S0 + (j // 2) * FR, 32)
        fc0 = pl.multiple_of((j % 2) * FC, 128)
        hs = []
        gs = {}

        def gate(k):
            xg = x_s[pl.ds(fr0, FR), :]
            c0 = pl.multiple_of(fc0 + k * 128, 128)
            gs[k] = _dot_nt(xg, wgt_s[pl.ds(c0, 128), :])

        def up(k):
            xg = x_s[pl.ds(fr0, FR), :]
            c0 = pl.multiple_of(fc0 + k * 128, 128)
            u = _dot_nt(xg, wut_s[pl.ds(c0, 128), :])
            hs.append((gelu(gs.pop(k)) * u).astype(BF16))

        def down(n):
            assert len(hs) == FC // 128
            hcat = jnp.concatenate(hs, axis=1)
            w = wd_s[pl.ds(fc0, FC), n * 128:(n + 1) * 128]
            bb_s[pl.ds(fr0, FR), n * 128:(n + 1) * 128] += _dot(hcat, w)

        def combine(iu):
            ru = pl.multiple_of(r0 + iu * 2 * SEG, 2 * SEG)
            xf = x_s[pl.ds(ru, 2 * SEG), :].astype(F32)
            z = jnp.sum(xf * gw_ref[...].astype(F32).reshape(1, D), axis=-1,
                        keepdims=True)
            gt = jax.nn.sigmoid(z)
            out_s[pl.ds(ru, 2 * SEG), :] = (
                gt * outs.pop(iu) + (1.0 - gt) * bb_s[pl.ds(ru, 2 * SEG), :]
            ).astype(out_s.dtype)

        outs = {}
        fills = dict(g=gate, u=up, d=down, c=combine)

        mem = mem_s[...]
        for iu in range(NU):
            ru = pl.multiple_of(r0 + iu * 2 * SEG, 2 * SEG)
            xf = x_s[pl.ds(ru, 2 * SEG), :].astype(F32)
            ha = jnp.concatenate([mem, xf[0:L]], axis=0).astype(BF16)
            acc_a = substep(ha, True, SCHED[2 * iu], fills)
            hb = jnp.concatenate([acc_a[0:M], xf[L:2 * SEG]],
                                 axis=0).astype(BF16)
            acc_b = substep(hb, False, SCHED[2 * iu + 1], fills)
            mem = acc_b[0:M]
            outs[iu] = jnp.concatenate(
                [acc_a[M:SEG], acc_b[L:L + M], acc_b[M:L]], axis=0)
        mem_s[...] = mem
        for iu in list(outs):
            combine(iu)
        pltpu.make_async_copy(out_s.at[pl.ds(r0, RB)],
                              out_hbm.at[pl.ds(r0, RB)], osem).start()
        return c

    jax.lax.fori_loop(0, n_it, seg_body, 0)
    pltpu.make_async_copy(out_s, out_hbm, osem).wait()


@jax.jit
def pallas_gated_mix__memory_aug_recurrent_mem_tr__glu_gated_geglu__prompt_kernel(
    A_x: jax.Array,
    A_mem0: jax.Array,
    A_Wq: jax.Array,
    A_Wk: jax.Array,
    A_Wv: jax.Array,
    A_Wo: jax.Array,
    A_seg_len: jax.Array,
    B_x: jax.Array,
    B_w_gate: jax.Array,
    B_w_up: jax.Array,
    B_w_down: jax.Array,
    gate_w: jax.Array,
):
    B, S, D = A_x.shape
    H, E = A_Wq.shape[1], A_Wq.shape[2]
    M = A_mem0.shape[1]
    DF = B_w_gate.shape[1]
    DFP = -(-DF // 256) * 256
    SEG = 32
    assert B == 1 and M == 8 and S == 2048 and D == 640 and H == 32

    kern = functools.partial(_kernel, S=S, D=D, H=H, E=E, M=M, SEG=SEG, DF=DF,
                             DFP=DFP)
    hbm = pl.BlockSpec(memory_space=pl.ANY)
    out = pl.pallas_call(
        kern,
        out_shape=jax.ShapeDtypeStruct((S, D), A_x.dtype),
        in_specs=[hbm] * 10,
        out_specs=hbm,
        scratch_shapes=[
            pltpu.VMEM((S, D), BF16),
            pltpu.VMEM((3 * D, H, E), BF16),
            pltpu.VMEM((H * E, D), BF16),
            pltpu.VMEM((DFP, D), BF16),
            pltpu.VMEM((DFP, D), BF16),
            pltpu.VMEM((DFP, D), BF16),
            pltpu.VMEM((3 * H * PH_ + 1024, E), U32),
            pltpu.VMEM((S, D), F32),
            pltpu.VMEM((5 * 256, DFP), F32),
            pltpu.VMEM((M, D), F32),
            pltpu.VMEM((3, H, M, E), F32),
            pltpu.VMEM((H, M, E), F32),
            pltpu.VMEM(((SEG + 2 * M) // 2, H * E), U32),
            pltpu.VMEM((S, D), BF16),
            pltpu.VMEM((M, D), BF16),
            pltpu.VMEM((D,), BF16),
            pltpu.SemaphoreType.DMA((12,)),
            pltpu.SemaphoreType.DMA((5,)),
            pltpu.SemaphoreType.DMA,
        ],
        compiler_params=pltpu.CompilerParams(
            vmem_limit_bytes=110 * 1024 * 1024),
    )(
        A_x.reshape(S, D), A_mem0.reshape(M, D), A_Wq, A_Wk, A_Wv,
        A_Wo.reshape(H * E, D), B_w_gate.T, B_w_up.T, B_w_down,
        gate_w,
    )
    return out.reshape(B, S, D)
```
